```python
import os as _os
_os.environ.setdefault("JAX_PLATFORMS", "cpu")
import jax
import jax.numpy as jnp

def _softmax(x, axis=-1):
    return jax.nn.softmax(x, axis=axis)
def _gelu(x):
    return jax.nn.gelu(x, approximate=True)
def _silu(x):
    return jax.nn.silu(x)
def _sigmoid(x):
    return jax.nn.sigmoid(x)
def _layernorm(x, axis=-1, eps=1e-5):
    m = jnp.mean(x, axis=axis, keepdims=True)
    v = jnp.var(x, axis=axis, keepdims=True)
    return (x - m) / jnp.sqrt(v + eps)
def _scatter_add(tgt, idx, src, axis=0):
    return tgt.at[idx].add(src)
def _segment_sum(src, seg, n):
    return jax.ops.segment_sum(src, seg, n)
class _Rng:
    def __init__(self, key):
        self._k = key
    def _next(self):
        self._k, sub = jax.random.split(self._k)
        return sub
    def normal(self, shape):
        return jax.random.normal(self._next(), shape, dtype=jnp.bfloat16)
    def randint(self, lo, hi, shape):
        return jax.random.randint(self._next(), shape, lo, hi, dtype=jnp.int32)
    def uniform(self, shape, lo=0.0, hi=1.0):
        return jax.random.uniform(self._next(), shape, jnp.bfloat16, lo, hi)
    def permutation(self, n):
        return jax.random.permutation(self._next(), n)


kernel_name = 'standalone__grn__sampling'

def setup_inputs():
    _rng = _Rng(jax.random.key(int.from_bytes(__import__("os").urandom(4), "little")))
    _w = (lambda a: (lambda t: t.astype(jnp.bfloat16) if jnp.issubdtype(t.dtype, jnp.floating) else t)(jnp.asarray(a)))
    B, S, D = 512, 32, 640
    return {
        "x": _w((lambda *s: _rng.normal(s) * 0.05)(B, S, D)),
        "g": _w((lambda *s: _rng.normal(s) * 0.1)(D) * 0.1),
        "b": _w((lambda *s: _rng.normal(s) * 0.1)(D) * 0.1),
    }

def reference(x, g, b):
    gx = jnp.sqrt((x * x).sum(axis=-2, keepdims=True))
    nx = gx / (gx.mean(axis=-1, keepdims=True) + 1e-6)
    return g * (x * nx) + b + x
```

```python
import jax
import jax.numpy as jnp
from jax import lax
import jax.experimental.pallas as pl
import jax.experimental.pallas.tpu as pltpu

_NREG = 8
_CH = 4
_NRS = 2
_EPS = 1e-6


@jax.jit
def pallas_standalone__grn__sampling_kernel(
    x: jax.Array,
    g: jax.Array,
    b: jax.Array,
):
    B, S, D = x.shape
    per = B // _NREG
    nch = per // _CH

    def kernel(x_hbm, g_hbm, b_hbm, o_hbm, xbuf, gbuf, bbuf, rsem, gsem, wsem):
        def rd(k):
            return pltpu.make_async_copy(
                x_hbm.at[:, pl.ds(k * _CH, _CH)],
                xbuf.at[:, pl.ds(k * _CH, _CH)],
                rsem.at[k % _NRS])

        def wr(j):
            return pltpu.make_async_copy(
                xbuf.at[:, pl.ds(j, 1)], o_hbm.at[:, pl.ds(j, 1)], wsem.at[0])

        gcp = pltpu.make_async_copy(g_hbm, gbuf, gsem.at[0])
        bcp = pltpu.make_async_copy(b_hbm, bbuf, gsem.at[1])
        rd(0).start()
        gcp.start()
        bcp.start()
        for k in range(1, _NRS):
            rd(k).start()
        gcp.wait()
        bcp.wait()
        g8 = jnp.broadcast_to(gbuf[...].astype(jnp.float32).reshape(1, D), (8, D))
        b8 = jnp.broadcast_to(bbuf[...].astype(jnp.float32).reshape(1, D), (8, D))
        sub = lax.broadcasted_iota(jnp.int32, (8, D), 0)
        m1 = (sub % 2) == 0
        m2 = (sub % 4) < 2
        m4 = sub < 4

        def comb(a, c, m, sh):
            return jnp.where(m, a, c) + pltpu.roll(jnp.where(m, c, a), sh, 0)

        def group(j):
            ps = []
            for r in range(_NREG):
                xr = xbuf[r, j].astype(jnp.float32)
                x2 = xr * xr
                ps.append((x2[0:8] + x2[8:16]) + (x2[16:24] + x2[24:32]))
            q = [comb(ps[2 * i], ps[2 * i + 1], m1, 1) for i in range(4)]
            rr = [comb(q[0], q[1], m2, 2), comb(q[2], q[3], m2, 2)]
            ss = comb(rr[0], rr[1], m4, 4)
            gx = jnp.sqrt(ss)
            m = jnp.sum(gx, axis=-1, keepdims=True) * (1.0 / D) + _EPS
            scale = g8 * (gx * (1.0 / m)) + 1.0
            for r in range(_NREG):
                xr = xbuf[r, j].astype(jnp.float32).reshape(S // 8, 8, D)
                sc = jnp.broadcast_to(scale[r:r + 1, :], (8, D))
                o = xr * sc[None] + b8[None]
                xbuf[r, j] = o.reshape(S, D).astype(xbuf.dtype)

        def compute(k):
            def body(i, c):
                group(k * _CH + i)
                return c
            lax.fori_loop(0, _CH, body, 0, unroll=2)

        def step(k, c):
            rd(k).wait()

            @pl.when(k + _NRS < nch)
            def _():
                rd(k + _NRS).start()

            compute(k)
            return c

        lax.fori_loop(0, nch - 1, step, 0)
        rd(nch - 1).wait()

        def issue(j, c):
            wr(j).start()
            return c

        lax.fori_loop(0, (nch - 1) * _CH, issue, 0)
        compute(nch - 1)
        for j in range((nch - 1) * _CH, per):
            wr(j).start()
        pltpu.make_async_copy(xbuf, o_hbm, wsem.at[0]).wait()

    xv = x.reshape(_NREG, per, S, D)
    out = pl.pallas_call(
        kernel,
        in_specs=[pl.BlockSpec(memory_space=pl.ANY)] * 3,
        out_specs=pl.BlockSpec(memory_space=pl.ANY),
        out_shape=jax.ShapeDtypeStruct(xv.shape, x.dtype),
        scratch_shapes=[
            pltpu.VMEM(xv.shape, x.dtype),
            pltpu.VMEM((D,), g.dtype),
            pltpu.VMEM((D,), b.dtype),
            pltpu.SemaphoreType.DMA((_NRS,)),
            pltpu.SemaphoreType.DMA((2,)),
            pltpu.SemaphoreType.DMA((1,)),
        ],
        compiler_params=pltpu.CompilerParams(vmem_limit_bytes=64 * 1024 * 1024),
    )(xv, g, b)
    return out.reshape(B, S, D)
```

```python
import jax
import jax.numpy as jnp
from jax import lax
import jax.experimental.pallas as pl
import jax.experimental.pallas.tpu as pltpu

_NREG = 8
_CH = 2
_NRS = 2
_EPS = 1e-6


@jax.jit
def pallas_standalone__grn__sampling_kernel(
    x: jax.Array,
    g: jax.Array,
    b: jax.Array,
):
    B, S, D = x.shape
    per = B // _NREG
    nm = (per - 2) // _CH

    def kernel(x_hbm, g_hbm, b_hbm, o_hbm, xbuf, gbuf, bbuf, rsem, wsem):
        def rdg(j0, n, k):
            return pltpu.make_async_copy(
                x_hbm.at[:, pl.ds(j0, n)], xbuf.at[:, pl.ds(j0, n)],
                rsem.at[k % _NRS])

        def rd(k):
            return rdg(k * _CH, _CH, k)

        def rd_static(k):
            if k < nm:
                return rd(k)
            if k < nm + 2:
                return rdg(nm * _CH + (k - nm), 1, k)
            return None

        def wr(j):
            return pltpu.make_async_copy(
                xbuf.at[:, pl.ds(j, 1)], o_hbm.at[:, pl.ds(j, 1)], wsem.at[0])

        gcp = pltpu.make_async_copy(g_hbm, gbuf, wsem.at[0])
        bcp = pltpu.make_async_copy(b_hbm, bbuf, wsem.at[0])
        rd(0).start()
        gcp.start()
        bcp.start()
        for k in range(1, _NRS):
            rd(k).start()
        gcp.wait()
        bcp.wait()
        g8 = jnp.broadcast_to(gbuf[...].astype(jnp.float32).reshape(1, D), (8, D))
        b8 = jnp.broadcast_to(bbuf[...].astype(jnp.float32).reshape(1, D), (8, D))
        sub = lax.broadcasted_iota(jnp.int32, (8, D), 0)
        m1 = (sub % 2) == 0
        m2 = (sub % 4) < 2
        m4 = sub < 4

        def comb(a, c, m, sh):
            return jnp.where(m, a, c) + pltpu.roll(jnp.where(m, c, a), sh, 0)

        def group(j):
            ps = []
            for r in range(_NREG):
                xr = xbuf[r, j].astype(jnp.float32)
                x2 = xr * xr
                ps.append((x2[0:8] + x2[8:16]) + (x2[16:24] + x2[24:32]))
            q = [comb(ps[2 * i], ps[2 * i + 1], m1, 1) for i in range(4)]
            rr = [comb(q[0], q[1], m2, 2), comb(q[2], q[3], m2, 2)]
            ss = comb(rr[0], rr[1], m4, 4)
            gx = jnp.sqrt(ss)
            m = jnp.sum(gx, axis=-1, keepdims=True) * (1.0 / D) + _EPS
            scale = g8 * (gx * (1.0 / m)) + 1.0
            for r in range(_NREG):
                xr = xbuf[r, j].astype(jnp.float32).reshape(S // 8, 8, D)
                sc = jnp.broadcast_to(scale[r:r + 1, :], (8, D))
                o = xr * sc[None] + b8[None]
                xbuf[r, j] = o.reshape(S, D).astype(xbuf.dtype)

        def compute(j0):
            for i in range(_CH):
                group(j0 + i)

        def step(k, c):
            rd(k).wait()
            rd(k + _NRS).start()
            compute(k * _CH)
            return c

        lax.fori_loop(0, nm - _NRS, step, 0)
        for k in range(nm - _NRS, nm - 1):
            rd(k).wait()
            rd_static(k + _NRS).start()
            compute(k * _CH)
        for k in (nm - 1, nm):
            rd_static(k).wait()
            nx = rd_static(k + _NRS)
            if nx is not None:
                nx.start()
        ndone = (nm - 1) * _CH

        def issue(j, c):
            wr(j).start()
            return c

        lax.fori_loop(0, ndone, issue, 0)
        rd_static(nm + 1).wait()

        def fin(j, c):
            group(j)
            wr(j).start()
            return c

        lax.fori_loop(ndone, per, fin, 0)
        pltpu.make_async_copy(xbuf, o_hbm, wsem.at[0]).wait()

    xv = x.reshape(_NREG, per, S, D)
    out = pl.pallas_call(
        kernel,
        in_specs=[pl.BlockSpec(memory_space=pl.ANY)] * 3,
        out_specs=pl.BlockSpec(memory_space=pl.ANY),
        out_shape=jax.ShapeDtypeStruct(xv.shape, x.dtype),
        scratch_shapes=[
            pltpu.VMEM(xv.shape, x.dtype),
            pltpu.VMEM((D,), g.dtype),
            pltpu.VMEM((D,), b.dtype),
            pltpu.SemaphoreType.DMA((_NRS,)),
            pltpu.SemaphoreType.DMA((1,)),
        ],
        compiler_params=pltpu.CompilerParams(vmem_limit_bytes=64 * 1024 * 1024),
    )(xv, g, b)
    return out.reshape(B, S, D)
```

```python
import jax
import jax.numpy as jnp
from jax import lax
import jax.experimental.pallas as pl
import jax.experimental.pallas.tpu as pltpu

_NREG = 8
_CH = 8
_UNROLL = 2
_EPS = 1e-6


@jax.jit
def pallas_standalone__grn__sampling_kernel(
    x: jax.Array,
    g: jax.Array,
    b: jax.Array,
):
    B, S, D = x.shape
    per = B // _NREG
    assert B == per * _NREG and per % _CH == 0 and per >= 2 * _CH
    assert S % 8 == 0 and _CH % _UNROLL == 0

    chunks = [(j, _CH) for j in range(0, per - _CH, _CH)]
    chunks += [(per - _CH, _CH - 1), (per - 1, 1)]
    nc = len(chunks)
    n_early = per - _CH

    def kernel(x_hbm, g_hbm, b_hbm, o_hbm, xbuf, gbuf, bbuf):
        def body(rsem, wsem):
            def rd(k):
                j0, n = chunks[k]
                return pltpu.make_async_copy(
                    x_hbm.at[:, pl.ds(j0, n)], xbuf.at[:, pl.ds(j0, n)],
                    rsem.at[k % 2])

            def wr(j):
                return pltpu.make_async_copy(
                    xbuf.at[:, pl.ds(j, 1)], o_hbm.at[:, pl.ds(j, 1)],
                    wsem.at[0])

            g_cp = pltpu.make_async_copy(g_hbm, gbuf, wsem.at[0])
            b_cp = pltpu.make_async_copy(b_hbm, bbuf, wsem.at[0])
            rd(0).start()
            g_cp.start()
            b_cp.start()
            rd(1).start()
            g_cp.wait()
            b_cp.wait()

            g8 = jnp.broadcast_to(
                gbuf[...].astype(jnp.float32).reshape(1, D), (8, D))
            b8 = jnp.broadcast_to(
                bbuf[...].astype(jnp.float32).reshape(1, D), (8, D))
            sub = lax.broadcasted_iota(jnp.int32, (8, D), 0)
            masks = ((sub % 2) == 0, (sub % 4) < 2, sub < 4)

            def merge(lo, hi, level):
                m = masks[level]
                return jnp.where(m, lo, hi) + pltpu.roll(
                    jnp.where(m, hi, lo), 1 << level, 0)

            def group(j):
                parts = []
                for r in range(_NREG):
                    xr = xbuf[r, j].astype(jnp.float32)
                    sq = xr * xr
                    rows = [sq[8 * i:8 * i + 8] for i in range(S // 8)]
                    while len(rows) > 1:
                        rows = [
                            rows[i] + rows[i + 1] if i + 1 < len(rows) else rows[i]
                            for i in range(0, len(rows), 2)
                        ]
                    parts.append(rows[0])
                for level in range(3):
                    parts = [
                        merge(parts[i], parts[i + 1], level)
                        for i in range(0, len(parts), 2)
                    ]
                gx = jnp.sqrt(parts[0])
                den = jnp.sum(gx, axis=-1, keepdims=True) * (1.0 / D) + _EPS
                scale = g8 * (gx * (1.0 / den)) + 1.0
                for r in range(_NREG):
                    xr = xbuf[r, j].astype(jnp.float32).reshape(S // 8, 8, D)
                    sc = jnp.broadcast_to(scale[r:r + 1, :], (8, D))
                    out = xr * sc[None] + b8[None]
                    xbuf[r, j] = out.reshape(S, D).astype(xbuf.dtype)

            def read_step(t, carry):
                j = t * _UNROLL
                for k in range(nc - 2):
                    @pl.when(j == chunks[k][0])
                    def _():
                        rd(k).wait()
                        rd(k + 2).start()
                for u in range(_UNROLL):
                    group(j + u)
                return carry

            lax.fori_loop(0, n_early // _UNROLL, read_step, 0)

            rd(nc - 2).wait()

            def write_step(j, carry):
                wr(j).start()
                return carry

            lax.fori_loop(0, n_early, write_step, 0)
            rd(nc - 1).wait()

            def tail_step(j, carry):
                group(j)
                wr(j).start()
                return carry

            lax.fori_loop(n_early, per, tail_step, 0)
            pltpu.make_async_copy(xbuf, o_hbm, wsem.at[0]).wait()

        pl.run_scoped(
            body,
            pltpu.SemaphoreType.DMA((2,)),
            pltpu.SemaphoreType.DMA((1,)),
        )

    xv = x.reshape(_NREG, per, S, D)
    out = pl.pallas_call(
        kernel,
        in_specs=[pl.BlockSpec(memory_space=pl.ANY)] * 3,
        out_specs=pl.BlockSpec(memory_space=pl.ANY),
        out_shape=jax.ShapeDtypeStruct(xv.shape, x.dtype),
        scratch_shapes=[
            pltpu.VMEM(xv.shape, x.dtype),
            pltpu.VMEM((D,), g.dtype),
            pltpu.VMEM((D,), b.dtype),
        ],
        compiler_params=pltpu.CompilerParams(vmem_limit_bytes=48 * 1024 * 1024),
    )(xv, g, b)
    return out.reshape(B, S, D)
```

```python
import jax
import jax.numpy as jnp
from jax import lax
import jax.experimental.pallas as pl
import jax.experimental.pallas.tpu as pltpu

_NREG = 8
_CH = 8
_UNROLL = 2
_WSPLIT = 2
_EPS = 1e-6


@jax.jit
def pallas_standalone__grn__sampling_kernel(
    x: jax.Array,
    g: jax.Array,
    b: jax.Array,
):
    B, S, D = x.shape
    per = B // _NREG
    assert B == per * _NREG and per % _CH == 0 and per >= 3 * _CH
    assert S % (16 * _WSPLIT) == 0 and _CH % _UNROLL == 0

    chunks = [(j, _CH) for j in range(0, per - _CH, _CH)]
    chunks += [(per - _CH, _CH - 1), (per - 1, 1)]
    nc = len(chunks)
    n_early = per - _CH

    def kernel(x_hbm, g_hbm, b_hbm, o_hbm, xbuf, gbuf, bbuf):
        def body(rsem, wsem):
            def rd(k):
                j0, n = chunks[k]
                return pltpu.make_async_copy(
                    x_hbm.at[:, pl.ds(j0, n)], xbuf.at[:, pl.ds(j0, n)],
                    rsem.at[k % 2])

            def start_write(j):
                rows = S // _WSPLIT
                for h in range(_WSPLIT):
                    sl = (slice(None), pl.ds(j, 1), pl.ds(h * rows, rows))
                    pltpu.make_async_copy(
                        xbuf.at[sl], o_hbm.at[sl], wsem.at[0]).start()

            g_cp = pltpu.make_async_copy(g_hbm, gbuf, wsem.at[0])
            b_cp = pltpu.make_async_copy(b_hbm, bbuf, wsem.at[0])
            rd(0).start()
            g_cp.start()
            b_cp.start()
            rd(1).start()
            g_cp.wait()
            b_cp.wait()

            g8 = jnp.broadcast_to(
                gbuf[...].astype(jnp.float32).reshape(1, D), (8, D))
            b8 = jnp.broadcast_to(
                bbuf[...].astype(jnp.float32).reshape(1, D), (8, D))
            sub = lax.broadcasted_iota(jnp.int32, (8, D), 0)
            masks = ((sub % 2) == 0, (sub % 4) < 2, sub < 4)

            def merge(lo, hi, level):
                m = masks[level]
                return jnp.where(m, lo, hi) + pltpu.roll(
                    jnp.where(m, hi, lo), 1 << level, 0)

            def group(j):
                parts = []
                for r in range(_NREG):
                    xr = xbuf[r, j].astype(jnp.float32)
                    sq = xr * xr
                    rows = [sq[8 * i:8 * i + 8] for i in range(S // 8)]
                    while len(rows) > 1:
                        rows = [
                            rows[i] + rows[i + 1] if i + 1 < len(rows) else rows[i]
                            for i in range(0, len(rows), 2)
                        ]
                    parts.append(rows[0])
                for level in range(3):
                    parts = [
                        merge(parts[i], parts[i + 1], level)
                        for i in range(0, len(parts), 2)
                    ]
                gx = jnp.sqrt(parts[0])
                den = jnp.sum(gx, axis=-1, keepdims=True) * (1.0 / D) + _EPS
                scale = g8 * (gx * (1.0 / den)) + 1.0
                for r in range(_NREG):
                    xr = xbuf[r, j].astype(jnp.float32).reshape(S // 8, 8, D)
                    sc = jnp.broadcast_to(scale[r:r + 1, :], (8, D))
                    out = xr * sc[None] + b8[None]
                    xbuf[r, j] = out.reshape(S, D).astype(xbuf.dtype)

            def read_step(t, carry):
                j = t * _UNROLL
                for k in range(nc - 2):
                    @pl.when(j == chunks[k][0])
                    def _():
                        rd(k).wait()
                        rd(k + 2).start()
                for u in range(_UNROLL):
                    group(j + u)
                return carry

            lax.fori_loop(0, n_early // _UNROLL, read_step, 0)

            rd(nc - 2).wait()

            def write_step(j, carry):
                start_write(j)
                return carry

            lax.fori_loop(0, _CH, write_step, 0)
            rd(nc - 1).wait()

            def tail_step(t, carry):
                group(n_early + t)
                start_write(_CH + t)
                return carry

            lax.fori_loop(0, _CH, tail_step, 0)
            lax.fori_loop(2 * _CH, per, write_step, 0)
            pltpu.make_async_copy(xbuf, o_hbm, wsem.at[0]).wait()

        pl.run_scoped(
            body,
            pltpu.SemaphoreType.DMA((2,)),
            pltpu.SemaphoreType.DMA((1,)),
        )

    xv = x.reshape(_NREG, per, S, D)
    out = pl.pallas_call(
        kernel,
        in_specs=[pl.BlockSpec(memory_space=pl.ANY)] * 3,
        out_specs=pl.BlockSpec(memory_space=pl.ANY),
        out_shape=jax.ShapeDtypeStruct(xv.shape, x.dtype),
        scratch_shapes=[
            pltpu.VMEM(xv.shape, x.dtype),
            pltpu.VMEM((D,), g.dtype),
            pltpu.VMEM((D,), b.dtype),
        ],
        compiler_params=pltpu.CompilerParams(vmem_limit_bytes=48 * 1024 * 1024),
    )(xv, g, b)
    return out.reshape(B, S, D)
```
